```python
import os as _os
_os.environ.setdefault("JAX_PLATFORMS", "cpu")
import jax
import jax.numpy as jnp

def _softmax(x, axis=-1):
    return jax.nn.softmax(x, axis=axis)
def _gelu(x):
    return jax.nn.gelu(x, approximate=True)
def _silu(x):
    return jax.nn.silu(x)
def _sigmoid(x):
    return jax.nn.sigmoid(x)
def _layernorm(x, axis=-1, eps=1e-5):
    m = jnp.mean(x, axis=axis, keepdims=True)
    v = jnp.var(x, axis=axis, keepdims=True)
    return (x - m) / jnp.sqrt(v + eps)
def _scatter_add(tgt, idx, src, axis=0):
    return tgt.at[idx].add(src)
def _segment_sum(src, seg, n):
    return jax.ops.segment_sum(src, seg, n)
class _Rng:
    def __init__(self, key):
        self._k = key
    def _next(self):
        self._k, sub = jax.random.split(self._k)
        return sub
    def normal(self, shape):
        return jax.random.normal(self._next(), shape, dtype=jnp.bfloat16)
    def randint(self, lo, hi, shape):
        return jax.random.randint(self._next(), shape, lo, hi, dtype=jnp.int32)
    def uniform(self, shape, lo=0.0, hi=1.0):
        return jax.random.uniform(self._next(), shape, jnp.bfloat16, lo, hi)
    def permutation(self, n):
        return jax.random.permutation(self._next(), n)


kernel_name = 'gated_mix__mha_block_cached__swiglu_ffn__decode'

def setup_inputs():
    _rng = _Rng(jax.random.key(int.from_bytes(__import__("os").urandom(4), "little")))
    _w = (lambda a: (lambda t: t.astype(jnp.bfloat16) if jnp.issubdtype(t.dtype, jnp.floating) else t)(jnp.asarray(a)))
    def _A_setup():
        B, Sq, D = 4, 1, 512
        H, Sk, Dh = 32, 4096, 128
        return {
            "x": _w((lambda *s: _rng.normal(s) * 0.05)(B, Sq, D)),
            "k_cache": _w((lambda *s: _rng.normal(s) * 3.2)(B, H, Sk, Dh)),
            "v_cache": _w((lambda *s: _rng.normal(s) * 0.4)(B, H, Sk, Dh)),
            "wq": _w((lambda *s: _rng.normal(s) * 3.2)(D, H * Dh) * (D ** -0.5)),
            "wo": _w((lambda *s: _rng.normal(s) * 0.4)(H * Dh, D) * ((H * Dh) ** -0.5)),
        }
    _A_in = _A_setup()

    def _B_setup():
        B, S, D, F = 4, 1, 512, 1376
        return {
            "x": _w((lambda *s: _rng.normal(s) * 0.05)(B, S, D)),
            "w_gate": _w((lambda *s: _rng.normal(s) * 0.05)(D, F)),
            "w_up": _w((lambda *s: _rng.normal(s) * 0.05)(D, F)),
            "w_down": _w((lambda *s: _rng.normal(s) * 0.05)(F, D)),
        }
    _B_in = _B_setup()

    return {
        "A_x": _A_in["x"],
        "A_k_cache": _A_in["k_cache"],
        "A_v_cache": _A_in["v_cache"],
        "A_wq": _A_in["wq"],
        "A_wo": _A_in["wo"],
        "B_x": _B_in["x"],
        "B_w_gate": _B_in["w_gate"],
        "B_w_up": _B_in["w_up"],
        "B_w_down": _B_in["w_down"],
        "gate_w": _w((lambda *s: _rng.normal(s) * 0.05)(512) * 16.0),
    }

def reference(A_x, A_k_cache, A_v_cache, A_wq, A_wo, B_x, B_w_gate, B_w_up, B_w_down, gate_w):
    def _A_ref(x, k_cache, v_cache, wq, wo):
        B, Sq, D = x.shape
        H, Dh = 32, 128
        q = (lambda x, *d: x.transpose(*d))((x @ wq).reshape(B, Sq, H, Dh), 0, 2, 1, 3)
        scores = jnp.einsum("bhqd,bhkd->bhqk", q, k_cache) * (Dh ** -0.5)
        p = _softmax(scores, axis=-1)
        o = jnp.einsum("bhqk,bhkd->bhqd", p, v_cache)
        return (lambda x, *d: x.transpose(*d))(o, 0, 2, 1, 3).reshape(B, Sq, H * Dh) @ wo

    def _B_ref(x, w_gate, w_up, w_down):
        g = _silu(x @ w_gate)
        u = x @ w_up
        return (g * u) @ w_down

    x = A_x
    g = _sigmoid((x * gate_w).sum(-1, keepdims=True))
    a = _A_ref(x, A_k_cache, A_v_cache, A_wq, A_wo)
    b = _B_ref(x, B_w_gate, B_w_up, B_w_down)
    return g * a + (1 - g) * b
```

```python
import functools

import jax
import jax.numpy as jnp
import numpy as np
from jax import lax
from jax.experimental import pallas as pl
from jax.experimental.pallas import tpu as pltpu

B, D, H, SK, DH, F = 4, 512, 32, 4096, 128, 1376
NS = 8
HG = H // 2
CH = 128
WR = 32
NT = (((1,), (1,)), ((), ()))


def make(nper=2, depth=4, nochecks=True, wq_mode=16, compute=True):
    C = nper * CH
    RPH = SK // C
    NR = HG * RPH
    G = 2 * NS * nper
    WO_DESC = H * DH // WR
    assert WO_DESC % G == 0 and WO_DESC // G <= depth
    f32, bf16 = jnp.float32, jnp.bfloat16

    def kernel(x_hbm, k_hbm, v_hbm, wq_hbm, wo_hbm, wg_hbm, wu_hbm, wd_hbm, gw_hbm, out_hbm,
               x_v, gw_v, wq_v, wo_v, wg_v, wu_v, wd_v, kv_v, q_v, o_v, out_v,
               kv_sem, w_sem):
        X_S, GW_S, WQ_S, WO_S, WG_S, WU_S, OUT_S, WD_S = range(8)

        def start_round(r, slot):
            j, i = r // RPH, r % RPH
            for c in range(nper):
                row = pl.multiple_of(i * C + c * CH, CH)
                for b in range(B):
                    for t in range(2):
                        for a, src in enumerate((k_hbm, v_hbm)):
                            pltpu.make_async_copy(
                                src.at[b, j + HG * t, pl.ds(row, CH)],
                                kv_v.at[slot, a, 4 * t + b, pl.ds(c * CH, CH)],
                                kv_sem.at[slot]).start(priority=a)

        def wait_all(ref, sem):
            pltpu.make_async_copy(ref, ref, sem).wait()

        def start_rows(src, dst, row, sem, prio):
            pltpu.make_async_copy(src.at[pl.ds(row, WR)], dst.at[pl.ds(row, WR)], sem).start(priority=prio)

        pltpu.make_async_copy(x_hbm, x_v, w_sem.at[X_S]).start()
        pltpu.make_async_copy(gw_hbm, gw_v, w_sem.at[GW_S]).start(priority=1)

        def wq_issue(i, carry):
            for m in range(8):
                if wq_mode == 16:
                    row = pl.multiple_of(m * 64 + (i // 4) * 16, 16)
                    col = pl.multiple_of((i % 4) * 1024, 1024)
                    sl = (pl.ds(row, 16), pl.ds(col, 1024))
                else:
                    row = pl.multiple_of(m * 64 + (i // 2) * 8, 8)
                    col = pl.multiple_of((i % 2) * 2048, 2048)
                    sl = (pl.ds(row, 8), pl.ds(col, 2048))
                pltpu.make_async_copy(wq_hbm.at[sl], wq_v.at[sl], w_sem.at[WQ_S]).start(priority=m % 2)
            return carry
        lax.fori_loop(0, 16, wq_issue, 0)

        def first_rounds(r, carry):
            start_round(r, r)
            return carry
        lax.fori_loop(0, depth, first_rounds, 0)

        wait_all(x_v, w_sem.at[X_S])
        wait_all(gw_v, w_sem.at[GW_S])
        wait_all(wq_v, w_sem.at[WQ_S])

        x4 = x_v[...].astype(f32)
        x8f = jnp.concatenate([x4, x4], axis=0)
        x8 = x8f.astype(bf16)
        row = lax.broadcasted_iota(jnp.int32, (NS, DH), 0)

        def q_proj(j, carry):
            lo = jnp.dot(x8, wq_v[:, pl.ds(pl.multiple_of(j * DH, DH), DH)], preferred_element_type=f32)
            hi = jnp.dot(x8, wq_v[:, pl.ds(pl.multiple_of((j + HG) * DH, DH), DH)], preferred_element_type=f32)
            q_v[j] = jnp.where(row < B, lo, hi)
            return carry
        lax.fori_loop(0, HG, q_proj, 0)

        rowc = lax.broadcasted_iota(jnp.int32, (NS, C), 0)

        def head_group(j, carry):
            q = q_v[j].astype(bf16)

            def one_round(i, state):
                m_prev, l_prev, acc = state
                r = j * RPH + i
                slot = r % depth
                wait_all(kv_v.at[slot], kv_sem.at[slot])
                if compute:
                    s = None
                    for n in range(NS):
                        sn = lax.dot_general(q, kv_v[slot, 0, n], NT, preferred_element_type=f32)
                        s = sn if s is None else jnp.where(rowc == n, sn, s)
                    s = s * (DH ** -0.5)
                    m_new = jnp.maximum(m_prev, jnp.max(s, axis=1, keepdims=True))
                    alpha = jnp.exp(m_prev - m_new)
                    p = jnp.exp(s - m_new)
                    psum = p[:, 0:DH]
                    for c in range(1, nper):
                        psum = psum + p[:, c * DH:(c + 1) * DH]
                    l_new = alpha * l_prev + psum
                    pb = p.astype(bf16)
                    pv = None
                    for n in range(NS):
                        on = jnp.dot(pb, kv_v[slot, 1, n], preferred_element_type=f32)
                        pv = on if pv is None else jnp.where(row == n, on, pv)
                    state = (m_new, l_new, alpha * acc + pv)

                @pl.when(r + depth < NR)
                def _():
                    start_round(r + depth, slot)

                @pl.when(jnp.logical_and(r + depth >= NR, r + depth < NR + WO_DESC // G))
                def _():
                    base = (r + depth - NR) * (G // 8)
                    for c in range(G // 8):
                        for m in range(8):
                            start_rows(wo_hbm, wo_v, pl.multiple_of(m * 512 + (base + c) * WR, WR),
                                       w_sem.at[WO_S], m % 2)
                return state

            init = (jnp.full((NS, 1), np.finfo(np.float32).min, f32),
                    jnp.zeros((NS, DH), f32), jnp.zeros((NS, DH), f32))
            _, l, acc = lax.fori_loop(0, RPH, one_round, init)
            o_v[j] = acc / jnp.sum(l, axis=1, keepdims=True)
            return carry
        lax.fori_loop(0, HG, head_group, 0)

        NF = F // WR

        def gu_issue(i, carry):
            rw = pl.multiple_of(((i * 16) % NF) * WR, WR)
            start_rows(wg_hbm, wg_v, rw, w_sem.at[WG_S], 0)
            start_rows(wu_hbm, wu_v, rw, w_sem.at[WU_S], 1)
            return carry
        lax.fori_loop(0, NF, gu_issue, 0)

        wait_all(wo_v, w_sem.at[WO_S])

        def o_proj(j, a):
            o = o_v[j].astype(bf16)
            lo = jnp.dot(o, wo_v[pl.ds(pl.multiple_of(j * DH, DH), DH), :], preferred_element_type=f32)
            hi = jnp.dot(o, wo_v[pl.ds(pl.multiple_of((j + HG) * DH, DH), DH), :], preferred_element_type=f32)
            return a[0] + lo, a[1] + hi
        z = jnp.zeros((NS, D), f32)
        a_lo, a_hi = lax.fori_loop(0, HG, o_proj, (z, z))
        attn = a_lo[0:B] + a_hi[B:NS]

        pieces = [(0, 512), (512, 512), (1024, 256), (1280, 96)]
        n = 0
        for pi, (r0, nr) in enumerate(pieces):
            for rw in range(r0, r0 + nr, WR):
                start_rows(wd_hbm, wd_v, rw, w_sem.at[WD_S + pi], n % 2)
                n += 1

        gw = gw_v[...].astype(f32)
        gl = x4[:, 0:DH] * gw[0:1]
        for c in range(1, D // DH):
            gl = gl + x4[:, c * DH:(c + 1) * DH] * gw[c:c + 1]
        gate = jax.nn.sigmoid(jnp.sum(gl, axis=1, keepdims=True))

        wait_all(wg_v, w_sem.at[WG_S])
        wait_all(wu_v, w_sem.at[WU_S])
        hs = []
        for (r0, nr) in pieces:
            g = lax.dot_general(x8, wg_v[pl.ds(r0, nr), :], NT, preferred_element_type=f32)
            u = lax.dot_general(x8, wu_v[pl.ds(r0, nr), :], NT, preferred_element_type=f32)
            hs.append((g * jax.nn.sigmoid(g) * u).astype(bf16))
        ffn = None
        for pi, (r0, nr) in enumerate(pieces):
            wait_all(wd_v.at[pl.ds(r0, nr)], w_sem.at[WD_S + pi])
            y = jnp.dot(hs[pi], wd_v[pl.ds(r0, nr), :], preferred_element_type=f32)
            ffn = y if ffn is None else ffn + y
        out_v[...] = (gate * attn + (1.0 - gate) * ffn[0:B]).astype(out_v.dtype)
        cp = pltpu.make_async_copy(out_v, out_hbm, w_sem.at[OUT_S])
        cp.start()
        cp.wait()

    def f(A_x, A_k_cache, A_v_cache, A_wq, A_wo, B_x, B_w_gate, B_w_up, B_w_down, gate_w):
        hbm = pl.BlockSpec(memory_space=pltpu.HBM)
        out = pl.pallas_call(
            kernel,
            out_shape=jax.ShapeDtypeStruct((B, D), A_x.dtype),
            in_specs=[hbm] * 9,
            out_specs=hbm,
            scratch_shapes=[
                pltpu.VMEM((B, D), bf16), pltpu.VMEM((D // DH, DH), bf16),
                pltpu.VMEM((D, H * DH), bf16), pltpu.VMEM((H * DH, D), bf16),
                pltpu.VMEM((F, D), bf16), pltpu.VMEM((F, D), bf16), pltpu.VMEM((F, D), bf16),
                pltpu.VMEM((depth, 2, NS, C, DH), bf16),
                pltpu.VMEM((HG, NS, DH), f32), pltpu.VMEM((HG, NS, DH), f32),
                pltpu.VMEM((B, D), A_x.dtype),
                pltpu.SemaphoreType.DMA((depth,)), pltpu.SemaphoreType.DMA((11,)),
            ],
            compiler_params=pltpu.CompilerParams(
                vmem_limit_bytes=100 * 2**20,
                disable_bounds_checks=nochecks, disable_semaphore_checks=nochecks),
        )(A_x.reshape(B, D), A_k_cache, A_v_cache, A_wq, A_wo,
          B_w_gate.T, B_w_up.T, B_w_down, gate_w.reshape(D // DH, DH))
        return out.reshape(B, 1, D)
    return f


@jax.jit
def pallas_gated_mix__mha_block_cached__swiglu_ffn__decode_kernel(
    A_x, A_k_cache, A_v_cache, A_wq, A_wo, B_x, B_w_gate, B_w_up, B_w_down, gate_w):
    return make(1, 8, wq_mode=8)(A_x, A_k_cache, A_v_cache, A_wq, A_wo, B_x, B_w_gate, B_w_up, B_w_down, gate_w)
```

```python
import contextlib

import jax
import jax.numpy as jnp
import numpy as np
from jax import lax
from jax.experimental import pallas as pl
from jax.experimental.pallas import tpu as pltpu

B, D, H, SK, DH, F = 4, 512, 32, 4096, 128, 1376
NS = 8
HG = H // 2
CH = 128
NT = (((1,), (1,)), ((), ()))
FH = F // 2


def make(depth=9, nochecks=True, kv_mode='m2', korder=(0, 3, 1, 2), vorder=(0, 3, 1, 2), hpos=2,
         wq_mode='m2', wq_perm=(64, 32, 1, 2, 4, 8, 16), f_mode='m2', f_mul=21, f_arr='gud',
         wo_mode='m2', wo_map=lambda e, n: (e + 8 * (n % 2), n // 2), wo_ord=lambda p: p // 2 + 8 * (p % 2), wo_gp=1, scopes=False, flags=None, order='fq',
         ffn_pieces=((0, 512), (512, 512), (1024, 352)), small_first=True, dst_contig=True, imul=1):
    RPH = SK // CH
    NR = HG * RPH
    assert depth >= 8 and sorted(wq_perm) == [1, 2, 4, 8, 16, 32, 64]
    NP = HG // wo_gp
    modes = dict(c128='cc', m2='mm', mix='cm', mix2='mc')[kv_mode]
    f32, bf16 = jnp.float32, jnp.bfloat16

    def scope(name):
        return jax.named_scope(name) if scopes else contextlib.nullcontext()

    def xor_bits(perm, n, lo, hi):
        v = 0
        for i in range(lo, hi):
            v = v ^ (((n >> (i - lo)) & 1) * perm[i])
        return v

    def kernel(x_hbm, k_hbm, v_hbm, wq_hbm, wo_hbm, wg_hbm, wu_hbm, wd_hbm, gw_hbm, out_hbm,
               x_v, gw_v, wq_v, wo_v, wg_v, wu_v, wd_v, k_v, v_v, o_v, out_v,
               kv_sem, w_sem, wo_sem):
        X_S, GW_S, WQ_S, WG_S, WU_S, WD_S, OUT_S = range(7)
        kv_v = (k_v, v_v)

        def start_round(r, slot):
            j, i = r // RPH, r % RPH
            if hpos == 2:
                seq = [(n, h) for h in range(2) for n in range(B)]
            elif hpos == 1:
                seq = [(2 * n1 + n0, h) for n1 in range(2) for h in range(2) for n0 in range(2)]
            else:
                seq = [(n, h) for n in range(B) for h in range(2)]
            ii = (i * imul) % RPH if imul != 1 else i
            for d, (n, h) in enumerate(seq):
                for a, src in enumerate((k_hbm, v_hbm)):
                    if modes[a] == 'c':
                        b, t = divmod(d, 2)
                        pltpu.make_async_copy(
                            src.at[b, t, j, pl.ds(pl.multiple_of(ii * CH, CH), CH)], kv_v[a].at[slot, b, t],
                            kv_sem.at[slot]).start(priority=a)
                    else:
                        b = (korder, vorder)[a][n]
                        row = pl.multiple_of(ii * CH + h * (CH // 2), CH // 2)
                        pltpu.make_async_copy(
                            src.at[b, :, j, pl.ds(row, CH // 2)],
                            kv_v[a].at[slot, b, :, pl.ds(h * (CH // 2), CH // 2)],
                            kv_sem.at[slot]).start(priority=a)

        def wait_all(ref, sem):
            pltpu.make_async_copy(ref, ref, sem).wait()

        def start_w(src, dst, unit, sem, prio, mode):
            if mode == 'm2':
                sl = (slice(None), pl.ds(pl.multiple_of(unit * 16, 16), 16))
            else:
                sl = (unit % 2, pl.ds(pl.multiple_of((unit // 2) * 32, 32), 32))
            pltpu.make_async_copy(src.at[sl], dst.at[sl], sem).start(priority=prio)

        def start_small():
            pltpu.make_async_copy(x_hbm, x_v, w_sem.at[X_S]).start()
            pltpu.make_async_copy(gw_hbm, gw_v, w_sem.at[GW_S]).start(priority=1)
        if small_first:
            start_small()

        def wq_issue(i, carry):
            for m in range(8):
                n = xor_bits(wq_perm, i, 3, 7) ^ xor_bits(wq_perm, m, 0, 3)
                if wq_mode == 'm2':
                    sl = (slice(None), pl.ds(pl.multiple_of((n >> 2) * 8, 8), 8),
                          pl.ds(pl.multiple_of((n & 3) * 1024, 1024), 1024))
                else:
                    sl = (n >> 6, pl.ds(pl.multiple_of(((n & 63) >> 1) * 8, 8), 8),
                          pl.ds(pl.multiple_of((n & 1) * 2048, 2048), 2048))
                pltpu.make_async_copy(wq_hbm.at[sl], wq_v.at[sl], w_sem.at[WQ_S]).start(priority=m % 2)
            return carry

        NF = FH // 16
        ffn = dict(g=(wg_hbm, wg_v, WG_S), u=(wu_hbm, wu_v, WU_S), d=(wd_hbm, wd_v, WD_S))

        def ffn_issue(i, carry):
            u0 = (2 * i * f_mul) % NF
            u1 = ((2 * i + 1) * f_mul) % NF
            for c in f_arr:
                src, dst, s = ffn[c]
                start_w(src, dst, u0, w_sem.at[s], 0, 'm2')
                start_w(src, dst, u1, w_sem.at[s], 1, 'm2')
            return carry

        def first_rounds(r, carry):
            start_round(r, r)
            return carry

        for what in order:
            if what == 'q':
                with scope('wq_issue'):
                    lax.fori_loop(0, 16, wq_issue, 0)
            else:
                with scope('ffn_issue'):
                    lax.fori_loop(0, NF // 2, ffn_issue, 0)
                    last = ((NF - 1) * f_mul) % NF
                    for n, c in enumerate(f_arr):
                        src, dst, s = ffn[c]
                        start_w(src, dst, last, w_sem.at[s], n % 2, 'm2')
        if not small_first:
            start_small()
        with scope('first_rounds'):
            lax.fori_loop(0, depth, first_rounds, 0)

        wait_all(x_v, w_sem.at[X_S])
        wait_all(gw_v, w_sem.at[GW_S])
        wait_all(wg_v, w_sem.at[WG_S])
        wait_all(wu_v, w_sem.at[WU_S])
        wait_all(wd_v, w_sem.at[WD_S])
        wait_all(wq_v, w_sem.at[WQ_S])

        with scope('ffn'):
            x4 = x_v[...].astype(f32)
            x8 = jnp.concatenate([x4, x4], axis=0).astype(bf16)
            gw = gw_v[...].astype(f32)
            gl = x4[:, 0:DH] * gw[0:1]
            for c in range(1, D // DH):
                gl = gl + x4[:, c * DH:(c + 1) * DH] * gw[c:c + 1]
            gate = jax.nn.sigmoid(jnp.sum(gl, axis=1, keepdims=True))
            y = None
            for half in range(2):
                g = lax.dot_general(x8, wg_v[half], NT, preferred_element_type=f32)
                u = lax.dot_general(x8, wu_v[half], NT, preferred_element_type=f32)
                h = (g * jax.nn.sigmoid(g) * u).astype(bf16)
                yh = jnp.dot(h, wd_v[half], preferred_element_type=f32)
                y = yh if y is None else y + yh
            mix = (1.0 - gate) * y[0:B]

        row = lax.broadcasted_iota(jnp.int32, (NS, DH), 0)

        def tile(slot, a, n):
            return kv_v[a][slot, n % B, n // B]

        def attend(q, slot, state):
            m_prev, l_prev, acc = state
            with scope('r'):
                wait_all(k_v.at[slot], kv_sem.at[slot])
                wait_all(v_v.at[slot], kv_sem.at[slot])
            s = None
            for n in range(NS):
                sn = lax.dot_general(q, tile(slot, 0, n), NT, preferred_element_type=f32)
                s = sn if s is None else jnp.where(row == n, sn, s)
            s = s * (DH ** -0.5)
            m_new = jnp.maximum(m_prev, jnp.max(s, axis=1, keepdims=True))
            alpha = jnp.exp(m_prev - m_new)
            p = jnp.exp(s - m_new)
            l_new = alpha * l_prev + p
            pb = p.astype(bf16)
            pv = None
            for n in range(NS):
                on = jnp.dot(pb, tile(slot, 1, n), preferred_element_type=f32)
                pv = on if pv is None else jnp.where(row == n, on, pv)
            return m_new, l_new, alpha * acc + pv

        def head_group(j, carry):
            def q_of(head):
                cols = pl.ds(pl.multiple_of(head * DH, DH), DH)
                return (jnp.dot(x8[:, :D // 2], wq_v[0, :, cols], preferred_element_type=f32)
                        + jnp.dot(x8[:, D // 2:], wq_v[1, :, cols], preferred_element_type=f32))
            q = jnp.where(row < B, q_of(j), q_of(j + HG)).astype(bf16)

            def one_round(i, state):
                r = j * RPH + i
                slot = r % depth
                state = attend(q, slot, state)

                @pl.when(r + depth < NR)
                def _():
                    start_round(r + depth, slot)

                @pl.when(jnp.logical_and(r + depth >= NR, r + depth < NR + HG // 2))
                def _():
                    e = r + depth - NR
                    for n in range(16):
                        g, c = wo_map(e, n)
                        start_w(wo_hbm, wo_v, g * 8 + c, wo_sem.at[g // wo_gp], n % 2, wo_mode)
                return state

            init = (jnp.full((NS, 1), np.finfo(np.float32).min, f32),
                    jnp.zeros((NS, DH), f32), jnp.zeros((NS, DH), f32))
            _, l, acc = lax.fori_loop(0, RPH, one_round, init)
            o = acc / jnp.sum(l, axis=1, keepdims=True)
            o_v[0, j] = o
            o_v[1, j] = pltpu.roll(o, B, axis=0)
            return carry
        lax.fori_loop(0, HG, head_group, 0)

        def o_proj(pp, a):
            pi = wo_ord(pp)
            with scope('wo_wait'):
                wait_all(wo_v.at[:, pl.ds(0, wo_gp * DH)], wo_sem.at[pi])
            for u in range(wo_gp):
                j = pi * wo_gp + u
                for t in range(2):
                    o = o_v[t, j].astype(bf16)
                    w = wo_v[t, pl.ds(pl.multiple_of(j * DH, DH), DH), :]
                    a += jnp.dot(o, w, preferred_element_type=f32)
            return a
        attn = lax.fori_loop(0, NP, o_proj, jnp.zeros((NS, D), f32))
        out_v[...] = (gate * attn[0:B] + mix).astype(out_v.dtype)
        cp = pltpu.make_async_copy(out_v, out_hbm, w_sem.at[OUT_S])
        with scope('out'):
            cp.start()
            cp.wait()

    def f(A_x, A_k_cache, A_v_cache, A_wq, A_wo, B_x, B_w_gate, B_w_up, B_w_down, gate_w):
        hbm = pl.BlockSpec(memory_space=pltpu.HBM)
        out = pl.pallas_call(
            kernel,
            out_shape=jax.ShapeDtypeStruct((B, D), A_x.dtype),
            in_specs=[hbm] * 9,
            out_specs=hbm,
            scratch_shapes=[
                pltpu.VMEM((B, D), bf16), pltpu.VMEM((D // DH, DH), bf16),
                pltpu.VMEM((2, D // 2, H * DH), bf16), pltpu.VMEM((2, HG * DH, D), bf16),
                pltpu.VMEM((2, FH, D), bf16), pltpu.VMEM((2, FH, D), bf16), pltpu.VMEM((2, FH, D), bf16),
                pltpu.VMEM((depth, B, 2, CH, DH), bf16), pltpu.VMEM((depth, B, 2, CH, DH), bf16),
                pltpu.VMEM((2, HG, NS, DH), f32),
                pltpu.VMEM((B, D), A_x.dtype),
                pltpu.SemaphoreType.DMA((depth,)), pltpu.SemaphoreType.DMA((7,)), pltpu.SemaphoreType.DMA((NP,)),
            ],
            compiler_params=pltpu.CompilerParams(
                vmem_limit_bytes=100 * 2**20, flags=flags,
                disable_bounds_checks=nochecks, disable_semaphore_checks=nochecks),
        )(A_x.reshape(B, D), A_k_cache.reshape(B, 2, HG, SK, DH), A_v_cache.reshape(B, 2, HG, SK, DH),
          A_wq.reshape(2, D // 2, H * DH), A_wo.reshape(2, HG * DH, D),
          B_w_gate.T.reshape(2, FH, D), B_w_up.T.reshape(2, FH, D), B_w_down.reshape(2, FH, D),
          gate_w.reshape(D // DH, DH))
        return out.reshape(B, 1, D)
    return f


@jax.jit
def pallas_gated_mix__mha_block_cached__swiglu_ffn__decode_kernel(
    A_x, A_k_cache, A_v_cache, A_wq, A_wo, B_x, B_w_gate, B_w_up, B_w_down, gate_w):
    return make(kv_mode='c128')(A_x, A_k_cache, A_v_cache, A_wq, A_wo, B_x, B_w_gate, B_w_up, B_w_down, gate_w)
```

```python
import jax
import jax.experimental.pallas as pl
import jax.experimental.pallas.tpu as pltpu
import jax.numpy as jnp
import numpy as np
from jax import lax

B, D, H, SK, DH, F = 4, 512, 32, 4096, 128, 1376

HG = H // 2
NS = 2 * B
CH = 128
PIECE = CH // 2
BATCH_ORDER = ((0, 3, 1, 2), (2, 1, 3, 0))
ROUNDS_PER_GROUP = SK // CH
ROUNDS = HG * ROUNDS_PER_GROUP
DEPTH = 10
W_ROWS = 32
F_COPIES = F // W_ROWS
F_STEP = 16
WO_ROUNDS = HG // 2

_CONTRACT_LAST = (((1,), (1,)), ((), ()))


def _kernel(
    x_hbm, k_hbm, v_hbm, wq_hbm, wo_hbm, wg_hbm, wu_hbm, wd_hbm, gw_hbm,
    out_hbm,
    x_buf, gw_buf, wq_buf, wo_buf, wg_buf, wu_buf, wd_buf, kv_buf, o_buf, out_buf,
    x_sem, gw_sem, wq_sem, wg_sem, wu_sem, wd_sem, out_sem, kv_sems, wo_sems,
):
    f32, bf16 = jnp.float32, jnp.bfloat16

    def start(src, dst, sem, queue):
        pltpu.make_async_copy(src, dst, sem).start(priority=queue)

    def wait_filled(buf, sem):
        pltpu.make_async_copy(buf, buf, sem).wait()

    def start_round(r, slot):
        j, i = r // ROUNDS_PER_GROUP, r % ROUNDS_PER_GROUP
        for half in range(2):
            rows = pl.ds(pl.multiple_of(i * CH + half * PIECE, PIECE), PIECE)
            for n in range(B):
                for a, cache in enumerate((k_hbm, v_hbm)):
                    b = BATCH_ORDER[a][n]
                    start(cache.at[b, :, j, rows],
                          kv_buf.at[slot, a, b, :, pl.ds(half * PIECE, PIECE)],
                          kv_sems.at[slot], queue=a)

    def start_wo(e):
        for c in range(DH // 16):
            for t in range(2):
                j = e + t * WO_ROUNDS
                rows = pl.ds(pl.multiple_of(j * DH + c * 16, 16), 16)
                start(wo_hbm.at[:, rows], wo_buf.at[:, rows], wo_sems.at[j], queue=t)

    start(x_hbm, x_buf, x_sem, queue=0)
    start(gw_hbm, gw_buf, gw_sem, queue=1)

    @pl.loop(0, 16)
    def _(i):
        cols = pl.ds(pl.multiple_of((i % 2) * 2048, 2048), 2048)
        for m, part in enumerate((0, 4, 2, 6, 1, 5, 3, 7)):
            rows = pl.ds(pl.multiple_of(part * 64 + (i // 2) * 8, 8), 8)
            start(wq_hbm.at[rows, cols], wq_buf.at[rows, cols], wq_sem, queue=m % 2)

    ffn = ((wg_hbm, wg_buf, wg_sem), (wu_hbm, wu_buf, wu_sem), (wd_hbm, wd_buf, wd_sem))

    def start_ffn(hbm, buf, sem, n, queue):
        rows = pl.ds(pl.multiple_of((n * F_STEP % F_COPIES) * W_ROWS, W_ROWS), W_ROWS)
        start(hbm.at[rows], buf.at[rows], sem, queue)

    @pl.loop(0, F_COPIES // 2)
    def _(i):
        for w in ffn:
            start_ffn(*w, i, queue=0)
            start_ffn(*w, i + F_COPIES // 2, queue=1)

    last = pl.ds(((F_COPIES - 1) * F_STEP % F_COPIES) * W_ROWS, W_ROWS)
    for n, (hbm, buf, sem) in enumerate(ffn):
        start(hbm.at[last], buf.at[last], sem, queue=n % 2)

    @pl.loop(0, DEPTH)
    def _(r):
        start_round(r, r)

    wait_filled(x_buf, x_sem)
    wait_filled(gw_buf, gw_sem)
    wait_filled(wq_buf, wq_sem)
    for _, buf, sem in ffn:
        wait_filled(buf, sem)

    x = x_buf[...].astype(f32)
    x8 = jnp.concatenate([x, x], axis=0).astype(bf16)

    gw = gw_buf[...].astype(f32)
    xg = x[:, 0:DH] * gw[0:1]
    for c in range(1, D // DH):
        xg = xg + x[:, c * DH:(c + 1) * DH] * gw[c:c + 1]
    gate = jax.nn.sigmoid(jnp.sum(xg, axis=1, keepdims=True))

    ffn_out = jnp.zeros((NS, D), f32)
    for half in range(2):
        rows = pl.ds(half * (F // 2), F // 2)
        g = lax.dot_general(x8, wg_buf[rows, :], _CONTRACT_LAST, preferred_element_type=f32)
        u = lax.dot_general(x8, wu_buf[rows, :], _CONTRACT_LAST, preferred_element_type=f32)
        hidden = (g * jax.nn.sigmoid(g) * u).astype(bf16)
        ffn_out += jnp.dot(hidden, wd_buf[rows, :], preferred_element_type=f32)
    ffn_mix = (1.0 - gate) * ffn_out[0:B]

    stream = lax.broadcasted_iota(jnp.int32, (NS, DH), 0)

    def per_stream(matmul):
        out = matmul(0)
        for n in range(1, NS):
            out = jnp.where(stream == n, matmul(n), out)
        return out

    @pl.loop(0, HG)
    def _(j):
        def q_proj(head):
            cols = pl.ds(pl.multiple_of(head * DH, DH), DH)
            return jnp.dot(x8, wq_buf[:, cols], preferred_element_type=f32)

        q = jnp.where(stream < B, q_proj(j), q_proj(j + HG)).astype(bf16)

        def one_round(i, state):
            m_prev, l_prev, acc = state
            r = j * ROUNDS_PER_GROUP + i
            slot = r % DEPTH
            wait_filled(kv_buf.at[slot], kv_sems.at[slot])

            s = per_stream(lambda n: lax.dot_general(
                q, kv_buf[slot, 0, n % B, n // B], _CONTRACT_LAST, preferred_element_type=f32))
            s = s * (DH ** -0.5)
            m = jnp.maximum(m_prev, jnp.max(s, axis=1, keepdims=True))
            alpha = jnp.exp(m_prev - m)
            p = jnp.exp(s - m)
            p_bf16 = p.astype(bf16)
            pv = per_stream(lambda n: jnp.dot(
                p_bf16, kv_buf[slot, 1, n % B, n // B], preferred_element_type=f32))

            nxt = r + DEPTH

            @pl.when(nxt < ROUNDS)
            def _():
                start_round(nxt, slot)

            @pl.when(jnp.logical_and(nxt >= ROUNDS, nxt < ROUNDS + WO_ROUNDS))
            def _():
                start_wo(nxt - ROUNDS)

            return m, alpha * l_prev + p, alpha * acc + pv

        init = (
            jnp.full((NS, 1), np.finfo(np.float32).min, f32),
            jnp.zeros((NS, CH), f32),
            jnp.zeros((NS, DH), f32),
        )
        _, l, acc = lax.fori_loop(0, ROUNDS_PER_GROUP, one_round, init)
        o = acc / jnp.sum(l, axis=1, keepdims=True)
        o_buf[0, j] = o
        o_buf[1, j] = pltpu.roll(o, B, axis=0)

    def o_proj(n, acc):
        j = n // 2 + (n % 2) * WO_ROUNDS
        rows = pl.ds(pl.multiple_of(j * DH, DH), DH)
        wait_filled(wo_buf.at[:, rows], wo_sems.at[j])
        for t in range(2):
            acc += jnp.dot(o_buf[t, j].astype(bf16), wo_buf[t, rows, :],
                           preferred_element_type=f32)
        return acc

    attn = lax.fori_loop(0, HG, o_proj, jnp.zeros((NS, D), f32))
    out_buf[...] = (gate * attn[0:B] + ffn_mix).astype(out_buf.dtype)
    start(out_buf, out_hbm, out_sem, queue=0)
    pltpu.make_async_copy(out_buf, out_hbm, out_sem).wait()


@jax.jit
def pallas_gated_mix__mha_block_cached__swiglu_ffn__decode_kernel(
    A_x: jax.Array,
    A_k_cache: jax.Array,
    A_v_cache: jax.Array,
    A_wq: jax.Array,
    A_wo: jax.Array,
    B_x: jax.Array,
    B_w_gate: jax.Array,
    B_w_up: jax.Array,
    B_w_down: jax.Array,
    gate_w: jax.Array,
):
    del B_x
    assert A_x.shape == (B, 1, D) and A_k_cache.shape == A_v_cache.shape == (B, H, SK, DH)
    assert B_w_down.shape == (F, D) and DEPTH >= WO_ROUNDS

    bf16 = jnp.bfloat16
    hbm = pl.BlockSpec(memory_space=pltpu.HBM)
    dma_sem = pltpu.SemaphoreType.DMA
    out = pl.pallas_call(
        _kernel,
        out_shape=jax.ShapeDtypeStruct((B, D), A_x.dtype),
        in_specs=[hbm] * 9,
        out_specs=hbm,
        scratch_shapes=[
            pltpu.VMEM((B, D), bf16),
            pltpu.VMEM((D // DH, DH), bf16),
            pltpu.VMEM((D, H * DH), bf16),
            pltpu.VMEM((2, HG * DH, D), bf16),
            pltpu.VMEM((F, D), bf16),
            pltpu.VMEM((F, D), bf16),
            pltpu.VMEM((F, D), bf16),
            pltpu.VMEM((DEPTH, 2, B, 2, CH, DH), bf16),
            pltpu.VMEM((2, HG, NS, DH), jnp.float32),
            pltpu.VMEM((B, D), A_x.dtype),
            *[dma_sem(())] * 7,
            dma_sem((DEPTH,)),
            dma_sem((HG,)),
        ],
        compiler_params=pltpu.CompilerParams(
            vmem_limit_bytes=48 * 2**20,
            disable_bounds_checks=True,
            disable_semaphore_checks=True,
        ),
    )(
        A_x.reshape(B, D),
        A_k_cache.reshape(B, 2, HG, SK, DH),
        A_v_cache.reshape(B, 2, HG, SK, DH),
        A_wq,
        A_wo.reshape(2, HG * DH, D),
        B_w_gate.T,
        B_w_up.T,
        B_w_down,
        gate_w.reshape(D // DH, DH),
    )
    return out.reshape(B, 1, D)
```

```python
import jax
import jax.experimental.pallas as pl
import jax.experimental.pallas.tpu as pltpu
import jax.numpy as jnp
import numpy as np
from jax import lax

B, D, H, SK, DH, F = 4, 512, 32, 4096, 128, 1376

HG = H // 2
NS = 2 * B
CH = 128
ROUNDS_PER_GROUP = SK // CH
ROUNDS = HG * ROUNDS_PER_GROUP
DEPTH = 10
W_ROWS = 32
F_COPIES = F // W_ROWS
F_STEP = 16
WO_ROUNDS = HG // 2

_CONTRACT_LAST = (((1,), (1,)), ((), ()))


def _kernel(
    x_hbm, k_hbm, v_hbm, wq_hbm, wo_hbm, wg_hbm, wu_hbm, wd_hbm, gw_hbm,
    out_hbm,
    x_buf, gw_buf, wq_buf, wo_buf, wg_buf, wu_buf, wd_buf, kv_buf, o_buf, out_buf,
    x_sem, gw_sem, wq_sem, wg_sem, wu_sem, wd_sem, out_sem, kv_sems, wo_sems,
):
    f32, bf16 = jnp.float32, jnp.bfloat16

    def start(src, dst, sem, queue):
        pltpu.make_async_copy(src, dst, sem).start(priority=queue)

    def wait_filled(buf, sem):
        pltpu.make_async_copy(buf, buf, sem).wait()

    def start_round(r, slot):
        j, i = r // ROUNDS_PER_GROUP, r % ROUNDS_PER_GROUP
        rows = pl.ds(pl.multiple_of(i * CH, CH), CH)
        for b in range(B):
            for t in range(2):
                for a, cache in enumerate((k_hbm, v_hbm)):
                    start(cache.at[b, j + t * HG, rows], kv_buf.at[slot, a, t * B + b],
                          kv_sems.at[slot], queue=a)

    def start_wo(e):
        for c in range(DH // 16):
            for t in range(2):
                j = e + t * WO_ROUNDS
                rows = pl.ds(pl.multiple_of(j * DH + c * 16, 16), 16)
                start(wo_hbm.at[:, rows], wo_buf.at[:, rows], wo_sems.at[j], queue=t)

    start(x_hbm, x_buf, x_sem, queue=0)
    start(gw_hbm, gw_buf, gw_sem, queue=1)

    @pl.loop(0, 16)
    def _(i):
        cols = pl.ds(pl.multiple_of((i % 2) * 2048, 2048), 2048)
        for m, part in enumerate((0, 4, 2, 6, 1, 5, 3, 7)):
            rows = pl.ds(pl.multiple_of(part * 64 + (i // 2) * 8, 8), 8)
            start(wq_hbm.at[rows, cols], wq_buf.at[rows, cols], wq_sem, queue=m % 2)

    ffn = ((wg_hbm, wg_buf, wg_sem), (wu_hbm, wu_buf, wu_sem), (wd_hbm, wd_buf, wd_sem))

    def start_ffn(hbm, buf, sem, n, queue):
        rows = pl.ds(pl.multiple_of((n * F_STEP % F_COPIES) * W_ROWS, W_ROWS), W_ROWS)
        start(hbm.at[rows], buf.at[rows], sem, queue)

    @pl.loop(0, F_COPIES // 2)
    def _(i):
        for w in ffn:
            start_ffn(*w, i, queue=0)
            start_ffn(*w, i + F_COPIES // 2, queue=1)

    last = pl.ds(((F_COPIES - 1) * F_STEP % F_COPIES) * W_ROWS, W_ROWS)
    for n, (hbm, buf, sem) in enumerate(ffn):
        start(hbm.at[last], buf.at[last], sem, queue=n % 2)

    @pl.loop(0, DEPTH)
    def _(r):
        start_round(r, r)

    wait_filled(x_buf, x_sem)
    wait_filled(gw_buf, gw_sem)
    wait_filled(wq_buf, wq_sem)
    for _, buf, sem in ffn:
        wait_filled(buf, sem)

    x = x_buf[...].astype(f32)
    x8 = jnp.concatenate([x, x], axis=0).astype(bf16)

    gw = gw_buf[...].astype(f32)
    xg = x[:, 0:DH] * gw[0:1]
    for c in range(1, D // DH):
        xg = xg + x[:, c * DH:(c + 1) * DH] * gw[c:c + 1]
    gate = jax.nn.sigmoid(jnp.sum(xg, axis=1, keepdims=True))

    ffn_out = jnp.zeros((NS, D), f32)
    for half in range(2):
        rows = pl.ds(half * (F // 2), F // 2)
        g = lax.dot_general(x8, wg_buf[rows, :], _CONTRACT_LAST, preferred_element_type=f32)
        u = lax.dot_general(x8, wu_buf[rows, :], _CONTRACT_LAST, preferred_element_type=f32)
        hidden = (g * jax.nn.sigmoid(g) * u).astype(bf16)
        ffn_out += jnp.dot(hidden, wd_buf[rows, :], preferred_element_type=f32)
    ffn_mix = (1.0 - gate) * ffn_out[0:B]

    stream = lax.broadcasted_iota(jnp.int32, (NS, DH), 0)

    def per_stream(matmul):
        out = matmul(0)
        for n in range(1, NS):
            out = jnp.where(stream == n, matmul(n), out)
        return out

    @pl.loop(0, HG)
    def _(j):
        def q_proj(head):
            cols = pl.ds(pl.multiple_of(head * DH, DH), DH)
            return jnp.dot(x8, wq_buf[:, cols], preferred_element_type=f32)

        q = jnp.where(stream < B, q_proj(j), q_proj(j + HG)).astype(bf16)

        def one_round(i, state):
            m_prev, l_prev, acc = state
            r = j * ROUNDS_PER_GROUP + i
            slot = r % DEPTH
            wait_filled(kv_buf.at[slot], kv_sems.at[slot])

            s = per_stream(lambda n: lax.dot_general(
                q, kv_buf[slot, 0, n], _CONTRACT_LAST, preferred_element_type=f32))
            s = s * (DH ** -0.5)
            m = jnp.maximum(m_prev, jnp.max(s, axis=1, keepdims=True))
            alpha = jnp.exp(m_prev - m)
            p = jnp.exp(s - m)
            p_bf16 = p.astype(bf16)
            pv = per_stream(lambda n: jnp.dot(
                p_bf16, kv_buf[slot, 1, n], preferred_element_type=f32))

            nxt = r + DEPTH

            @pl.when(nxt < ROUNDS)
            def _():
                start_round(nxt, slot)

            @pl.when(jnp.logical_and(nxt >= ROUNDS, nxt < ROUNDS + WO_ROUNDS))
            def _():
                start_wo(nxt - ROUNDS)

            return m, alpha * l_prev + p, alpha * acc + pv

        init = (
            jnp.full((NS, 1), np.finfo(np.float32).min, f32),
            jnp.zeros((NS, CH), f32),
            jnp.zeros((NS, DH), f32),
        )
        _, l, acc = lax.fori_loop(0, ROUNDS_PER_GROUP, one_round, init)
        o = acc / jnp.sum(l, axis=1, keepdims=True)
        o_buf[0, j] = o
        o_buf[1, j] = pltpu.roll(o, B, axis=0)

    def o_proj(n, acc):
        j = n // 2 + (n % 2) * WO_ROUNDS
        rows = pl.ds(pl.multiple_of(j * DH, DH), DH)
        wait_filled(wo_buf.at[:, rows], wo_sems.at[j])
        for t in range(2):
            acc += jnp.dot(o_buf[t, j].astype(bf16), wo_buf[t, rows, :],
                           preferred_element_type=f32)
        return acc

    attn = lax.fori_loop(0, HG, o_proj, jnp.zeros((NS, D), f32))
    out_buf[...] = (gate * attn[0:B] + ffn_mix).astype(out_buf.dtype)
    start(out_buf, out_hbm, out_sem, queue=0)
    pltpu.make_async_copy(out_buf, out_hbm, out_sem).wait()


@jax.jit
def pallas_gated_mix__mha_block_cached__swiglu_ffn__decode_kernel(
    A_x: jax.Array,
    A_k_cache: jax.Array,
    A_v_cache: jax.Array,
    A_wq: jax.Array,
    A_wo: jax.Array,
    B_x: jax.Array,
    B_w_gate: jax.Array,
    B_w_up: jax.Array,
    B_w_down: jax.Array,
    gate_w: jax.Array,
):
    del B_x
    assert A_x.shape == (B, 1, D) and A_k_cache.shape == A_v_cache.shape == (B, H, SK, DH)
    assert B_w_down.shape == (F, D) and DEPTH >= WO_ROUNDS

    bf16 = jnp.bfloat16
    hbm = pl.BlockSpec(memory_space=pltpu.HBM)
    dma_sem = pltpu.SemaphoreType.DMA
    out = pl.pallas_call(
        _kernel,
        out_shape=jax.ShapeDtypeStruct((B, D), A_x.dtype),
        in_specs=[hbm] * 9,
        out_specs=hbm,
        scratch_shapes=[
            pltpu.VMEM((B, D), bf16),
            pltpu.VMEM((D // DH, DH), bf16),
            pltpu.VMEM((D, H * DH), bf16),
            pltpu.VMEM((2, HG * DH, D), bf16),
            pltpu.VMEM((F, D), bf16),
            pltpu.VMEM((F, D), bf16),
            pltpu.VMEM((F, D), bf16),
            pltpu.VMEM((DEPTH, 2, NS, CH, DH), bf16),
            pltpu.VMEM((2, HG, NS, DH), jnp.float32),
            pltpu.VMEM((B, D), A_x.dtype),
            *[dma_sem(())] * 7,
            dma_sem((DEPTH,)),
            dma_sem((HG,)),
        ],
        compiler_params=pltpu.CompilerParams(
            vmem_limit_bytes=48 * 2**20,
            disable_bounds_checks=True,
            disable_semaphore_checks=True,
        ),
    )(
        A_x.reshape(B, D),
        A_k_cache,
        A_v_cache,
        A_wq,
        A_wo.reshape(2, HG * DH, D),
        B_w_gate.T,
        B_w_up.T,
        B_w_down,
        gate_w.reshape(D // DH, DH),
    )
    return out.reshape(B, 1, D)
```
